```python
import os as _os
_os.environ.setdefault("JAX_PLATFORMS", "cpu")
import jax
import jax.numpy as jnp

def _softmax(x, axis=-1):
    return jax.nn.softmax(x, axis=axis)
def _gelu(x):
    return jax.nn.gelu(x, approximate=True)
def _silu(x):
    return jax.nn.silu(x)
def _sigmoid(x):
    return jax.nn.sigmoid(x)
def _layernorm(x, axis=-1, eps=1e-5):
    m = jnp.mean(x, axis=axis, keepdims=True)
    v = jnp.var(x, axis=axis, keepdims=True)
    return (x - m) / jnp.sqrt(v + eps)
def _scatter_add(tgt, idx, src, axis=0):
    return tgt.at[idx].add(src)
def _segment_sum(src, seg, n):
    return jax.ops.segment_sum(src, seg, n)
class _Rng:
    def __init__(self, key):
        self._k = key
    def _next(self):
        self._k, sub = jax.random.split(self._k)
        return sub
    def normal(self, shape):
        return jax.random.normal(self._next(), shape, dtype=jnp.bfloat16)
    def randint(self, lo, hi, shape):
        return jax.random.randint(self._next(), shape, lo, hi, dtype=jnp.int32)
    def uniform(self, shape, lo=0.0, hi=1.0):
        return jax.random.uniform(self._next(), shape, jnp.bfloat16, lo, hi)
    def permutation(self, n):
        return jax.random.permutation(self._next(), n)


kernel_name = 'concat_heads__ssm_conv_s4__linear_attn_block__prompt'

def setup_inputs():
    _rng = _Rng(jax.random.key(int.from_bytes(__import__("os").urandom(4), "little")))
    _w = (lambda a: (lambda t: t.astype(jnp.bfloat16) if jnp.issubdtype(t.dtype, jnp.floating) else t)(jnp.asarray(a)))
    def _A_setup():
        B, L, D, N = 1, 2048, 512, 128
        A_re = -jnp.exp((lambda *s: _rng.normal(s) * 0.1)(D, N))
        A_im = jnp.pi * (lambda *s: _rng.normal(s) * 0.1)(D, N)
        B_re = (lambda *s: _rng.normal(s) * 0.1)(D, N)
        B_im = (lambda *s: _rng.normal(s) * 0.1)(D, N)
        C_re = (lambda *s: _rng.normal(s) * 0.1)(D, N)
        C_im = (lambda *s: _rng.normal(s) * 0.1)(D, N)
        log_dt = (lambda *s: _rng.normal(s) * 0.1)(D) * 0.5 - 4.0
        Dskip = (lambda *s: _rng.normal(s) * 0.05)(D)
        return {
            "u": _w((lambda *s: _rng.normal(s) * 0.05)(B, L, D)),
            "A_re": _w(A_re),
            "A_im": _w(A_im),
            "B_re": _w(B_re),
            "B_im": _w(B_im),
            "C_re": _w(C_re),
            "C_im": _w(C_im),
            "log_dt": _w(log_dt),
            "Dskip": _w(Dskip),
        }
    _A_in = _A_setup()

    def _B_setup():
        B, S, D = 1, 2048, 512
        return {
            "x": _w((lambda *s: _rng.normal(s) * 0.05)(B, S, D)),
            "wqkv": _w((lambda *s: _rng.normal(s) * 0.4)(D, 3 * D)),
            "wo": _w((lambda *s: _rng.normal(s) * 0.05)(D, D)),
        }
    _B_in = _B_setup()

    return {
        "A_u": _A_in["u"],
        "A_A_re": _A_in["A_re"],
        "A_A_im": _A_in["A_im"],
        "A_B_re": _A_in["B_re"],
        "A_B_im": _A_in["B_im"],
        "A_C_re": _A_in["C_re"],
        "A_C_im": _A_in["C_im"],
        "A_log_dt": _A_in["log_dt"],
        "A_Dskip": _A_in["Dskip"],
        "B_x": _B_in["x"],
        "B_wqkv": _B_in["wqkv"],
        "B_wo": _B_in["wo"],
    }

def reference(A_u, A_A_re, A_A_im, A_B_re, A_B_im, A_C_re, A_C_im, A_log_dt, A_Dskip, B_x, B_wqkv, B_wo):
    def _A_ref(u, A_re, A_im, B_re, B_im, C_re, C_im, log_dt, Dskip):
        Bsz, L, D = u.shape
        dt = jnp.exp(log_dt)[:, None]
        A = A_re + 1j * A_im
        Bc = B_re + 1j * B_im
        Cc = C_re + 1j * C_im
        logdA = dt * A
        dB = dt * Bc
        l = (lambda x, dt: x.astype(dt))(jnp.arange(L), A_re.dtype)
        P = jnp.exp(logdA[:, :, None] * l[None, None, :])
        K = jnp.einsum("dn,dnl,dn->dl", Cc, P, dB).real
        L2 = 2 * L
        Kp = jnp.pad(K, ((0, 0), (0, L)))
        up = (lambda x, *d: x.transpose(*d))(u, 0, 2, 1)
        up = jnp.pad(up, ((0, 0), (0, 0), (0, L)))
        Kf = (lambda x, axes=(-2,-1): jnp.fft.rfft2(x.astype(jnp.float32), axes=axes))(Kp[:, None, :], axes=(-2, -1))
        Uf = (lambda x, axes=(-2,-1): jnp.fft.rfft2(x.astype(jnp.float32), axes=axes))(up[:, :, None, :], axes=(-2, -1))
        Yf = Uf * Kf[None, :, :, :]
        y = (lambda x, s, axes=(-2,-1): jnp.fft.irfft2(x, s=s, axes=axes).astype(jnp.bfloat16))(Yf, (1, L2), axes=(-2, -1))[:, :, 0, :L]
        y = (lambda x, *d: x.transpose(*d))(y, 0, 2, 1) + u * Dskip[None, None, :]
        return y

    def _B_ref(x, wqkv, wo):
        B, S, D = x.shape
        H = 32; Dh = D // H
        qkv = (lambda x, *d: x.transpose(*d))((x @ wqkv).reshape(B, S, 3, H, Dh), 2, 0, 3, 1, 4)
        q, k, v = qkv[0], qkv[1], qkv[2]
        phi = lambda t: jnp.where(t > 0, t + 1, jnp.exp(t)) + 1e-6
        pq, pk = phi(q), phi(k)
        kv = jnp.einsum("bhsd,bhse->bhde", pk, v)
        z = jnp.einsum("bhsd->bhd", pk)
        num = jnp.einsum("bhqd,bhde->bhqe", pq, kv)
        den = jnp.einsum("bhqd,bhd->bhq", pq, z)[..., None] + 1e-6
        o = num / den
        return (lambda x, *d: x.transpose(*d))(o, 0, 2, 1, 3).reshape(B, S, D) @ wo

    a = _A_ref(A_u, A_A_re, A_A_im, A_B_re, A_B_im, A_C_re, A_C_im, A_log_dt, A_Dskip)
    b = _B_ref(B_x, B_wqkv, B_wo)
    return jnp.concatenate([a, b], axis=-1)
```

```python
import jax
import jax.numpy as jnp
import numpy as np
import jax.experimental.pallas as pl
import jax.experimental.pallas.tpu as pltpu

F32, BF = jnp.float32, jnp.bfloat16


def _consts():
    k1 = np.arange(128)
    ang = -2 * np.pi * np.outer(k1 + 0.5, np.arange(128)) / 256
    f1 = np.stack([np.cos(ang), np.sin(ang)], 1).reshape(256, 128)
    m = np.zeros((32, 2, 16, 4, 16, 4, 2))
    k0 = np.arange(16)[:, None]
    t0 = np.arange(16)[None, :]
    for g in range(32):
        for j in range(4):
            a = -2 * np.pi * t0 * (4 * g + j + 0.5 + 256 * k0) / 4096
            c, s = np.cos(a), np.sin(a)
            m[g, 0, :, j, :, j, 0] = c
            m[g, 0, :, j, :, j, 1] = -s
            m[g, 1, :, j, :, j, 0] = s
            m[g, 1, :, j, :, j, 1] = c
    m = m.reshape(32, 128, 128)
    return f1, m, f1.T.copy(), m.transpose(0, 2, 1).copy()


QS = (list(range(8)) + [256 + x for x in (0, 2, 4, 6, 8)]
      + [b + x for b in (512, 768) for x in (0, 4, 8)]
      + [b + x for b in (1024, 1280, 1536, 1792) for x in (0, 8)])


def _rnd(l):
    st = 1 if l < 256 else 2 if l < 512 else 4 if l < 1024 else 8
    q, r = divmod(l, st)
    if 2 * r > st or (2 * r == st and q % 2):
        q += 1
    return q * st


def cmul(a, b):
    return a[0] * b[0] - a[1] * b[1], a[0] * b[1] + a[1] * b[0]


def dot(a, b):
    return jnp.dot(a, b, preferred_element_type=F32)


def kern(u_ref, are, aim, bre, bim, cre, cim, ldt, dsk, x_ref, wqkv, wo,
         f1, m2, f1t, m2t, o_ref, e0, e1, r_s, kt, uf, z, kf, pq):
    dt = jnp.exp(ldt[...].astype(F32)).astype(BF).astype(F32)
    xr = dt * are[...].astype(F32)
    xi = dt * aim[...].astype(F32)
    mag = jnp.exp(xr)
    a1 = (mag * jnp.cos(xi), mag * jnp.sin(xi))
    w = cmul((cre[...].astype(F32), cim[...].astype(F32)),
             (dt * bre[...].astype(F32), dt * bim[...].astype(F32)))
    pw = {1: a1}
    for k in range(1, 11):
        pw[2 ** k] = cmul(pw[2 ** (k - 1)], pw[2 ** (k - 1)])

    def put(ref, row, v, sgn):
        for ch in range(4):
            ref[:, ch * 32 + row, 0:128] = v[0][ch * 128:(ch + 1) * 128]
            ref[:, ch * 32 + row, 128:256] = sgn * v[1][ch * 128:(ch + 1) * 128]

    def power(cache, e):
        if e not in cache:
            hb = 1 << (e.bit_length() - 1)
            cache[e] = cmul(power(cache, e - hb), pw[hb])
        return cache[e]

    for ch in range(4):
        e1[:, ch * 32 + 24:ch * 32 + 32, :] = jnp.zeros((128, 8, 256), F32)
    c1 = {0: (jnp.ones_like(xr), jnp.zeros_like(xr))}
    for i, q in enumerate(QS):
        put(e1, i, power(c1, q), 1.0)
    c0 = {0: w}
    for i, e in enumerate((0, 128, 8, 136)):
        v = power(c0, e)
        e0[2 * i] = v[0]
        e0[2 * i + 1] = v[1]

    lane = jax.lax.broadcasted_iota(jnp.int32, (32, 128), 1) // 32

    def kg(g, c):
        l1 = e1[g]
        rows = []
        for ch in range(4):
            b = (l1[ch * 32:ch * 32 + 8, :128], l1[ch * 32:ch * 32 + 8, 128:])
            for _ in range(4):
                b = (b[0] * b[0] - b[1] * b[1], 2.0 * b[0] * b[1])
            d = pl.ds(ch * 128 + g, 1)
            for i in range(4):
                v = cmul(b, (e0[2 * i, d, :], e0[2 * i + 1, d, :]))
                rows.append(jnp.concatenate([v[0], -v[1]], 1))
        r = jax.lax.dot_general(l1.astype(BF), jnp.concatenate(rows, 0).astype(BF),
                                (((1,), (1,)), ((), ())), preferred_element_type=F32)
        s = r[0:32]
        for ch in range(1, 4):
            s = jnp.where(lane == ch, r[ch * 32:ch * 32 + 32], s)
        r_s[:, pl.ds(g, 1), :] = s.reshape(32, 1, 128)
        return c
    jax.lax.fori_loop(0, 128, kg, 0, unroll=4)
    for i in range(len(QS)):
        t = r_s[i].T
        for ch in range(4):
            kt[i, :, ch * 128:(ch + 1) * 128] = t[ch * 32:(ch + 1) * 32]

    def stage2(g):
        rows = pl.ds(pl.multiple_of(g * 8, 8), 8)
        return dot(m2[g], z[:, rows, :].reshape(128, 512).astype(BF))

    for t0 in range(16):
        par = t0 // 8
        km = jnp.concatenate(
            [kt[QS.index(_rnd(256 * b + t0) - 8 * par), 16 * par:16 * par + 16, :]
             for b in range(8)], axis=0)
        z[t0] = dot(f1[...], km.astype(BF))

    def s2k(g, c):
        kf[g] = stage2(g)
        return c
    jax.lax.fori_loop(0, 32, s2k, 0, unroll=2)

    for c in range(4):
        uf[c] = u_ref[:, c * 128:(c + 1) * 128].astype(F32)

    def ld(t0):
        return jnp.concatenate([uf[c, pl.ds(t0, 128, stride=16), :] for c in range(4)], 1)
    for t0 in range(16):
        z[t0] = dot(f1[...], ld(t0).astype(BF))

    def s2u(g, c):
        x = stage2(g)
        k = kf[g]
        y = cmul((x[:64], x[64:]), (k[:64], k[64:]))
        y = dot(m2t[g], jnp.concatenate(y, 0).astype(BF))
        z[:, pl.ds(pl.multiple_of(g * 8, 8), 8), :] = y.reshape(16, 8, 512)
        return c
    jax.lax.fori_loop(0, 32, s2u, 0, unroll=2)
    ds = dsk[...]
    for t0 in range(16):
        y = (dot(f1t[...], z[t0].astype(BF)) * (1.0 / 2048)).astype(BF).astype(F32)
        rows = pl.ds(t0, 128, stride=16)
        y = y + (ld(t0).astype(BF) * ds).astype(F32)
        for c in range(4):
            uf[c, rows, :] = y[:, c * 128:(c + 1) * 128]
    for c in range(4):
        o_ref[:, c * 128:(c + 1) * 128] = uf[c].astype(BF)

    def phi(t):
        return (jnp.where(t > 0, t + 1, jnp.exp(t)) + 1e-6).astype(BF)
    g = jnp.zeros((512, 512), F32)
    zz = jnp.zeros((1, 512), F32)
    for i in range(4):
        rs = slice(i * 512, (i + 1) * 512)
        xb = x_ref[rs, :]
        pq[rs, :] = phi(dot(xb, wqkv[:, 0:512]))
        pk = phi(dot(xb, wqkv[:, 512:1024]))
        zz = zz + jnp.sum(pk.astype(F32), 0, keepdims=True)
        g = g + jax.lax.dot_general(pk, xb, (((0,), (0,)), ((), ())),
                                    preferred_element_type=F32)
    kv = dot(g.astype(BF), wqkv[:, 1024:1536])
    bd = (jax.lax.broadcasted_iota(jnp.int32, (512, 512), 0) // 16
          == jax.lax.broadcasted_iota(jnp.int32, (512, 512), 1) // 16)
    mm = dot(jnp.where(bd, kv, 0.0).astype(BF), wo[...]).astype(BF)
    zm = jnp.where(bd, zz, 0.0).astype(BF)
    for i in range(4):
        rs = slice(i * 512, (i + 1) * 512)
        p = pq[rs, :]
        den = jnp.concatenate(
            [jax.lax.dot_general(p[:, j * 128:(j + 1) * 128],
                                 zm[j * 128:(j + 1) * 128, j * 128:(j + 1) * 128],
                                 (((1,), (1,)), ((), ())), preferred_element_type=F32)
             for j in range(4)], 1) + 1e-6
        o_ref[rs, 512:1024] = dot((p.astype(F32) / den).astype(BF), mm).astype(BF)


@jax.jit
def pallas_concat_heads__ssm_conv_s4__linear_attn_block__prompt_kernel(
    A_u, A_A_re, A_A_im, A_B_re, A_B_im, A_C_re, A_C_im, A_log_dt, A_Dskip,
    B_x, B_wqkv, B_wo,
):
    cs = [jnp.asarray(c.astype(np.float32)).astype(BF) for c in _consts()]
    V = pltpu.VMEM
    out = pl.pallas_call(
        kern,
        out_shape=jax.ShapeDtypeStruct((2048, 1024), BF),
        scratch_shapes=[V((8, 512, 128), F32), V((128, 128, 256), F32),
                        V((32, 128, 128), F32), V((27, 32, 512), F32),
                        V((4, 2048, 128), F32), V((16, 256, 512), F32),
                        V((32, 128, 512), F32), V((2048, 512), BF)],
        compiler_params=pltpu.CompilerParams(vmem_limit_bytes=120 << 20),
    )(A_u.reshape(2048, 512), A_A_re, A_A_im, A_B_re, A_B_im, A_C_re, A_C_im,
      A_log_dt.reshape(512, 1), A_Dskip.reshape(1, 512), B_x.reshape(2048, 512),
      B_wqkv, B_wo, *cs)
    return out.reshape(1, 2048, 1024)
```
